```python
import jax
import jax.numpy as jnp

def _softmax(x, axis=-1):
    return jax.nn.softmax(x, axis=axis)
def _gelu(x):
    return jax.nn.gelu(x, approximate=True)
def _silu(x):
    return jax.nn.silu(x)
def _sigmoid(x):
    return jax.nn.sigmoid(x)
def _layernorm(x, axis=-1, eps=1e-5):
    m = jnp.mean(x, axis=axis, keepdims=True)
    v = jnp.var(x, axis=axis, keepdims=True)
    return (x - m) / jnp.sqrt(v + eps)
def _scatter_add(tgt, idx, src, axis=0):
    return tgt.at[idx].add(src)
def _segment_sum(src, seg, n):
    return jax.ops.segment_sum(src, seg, n)
class _Rng:
    def __init__(self, key):
        self._k = key
    def _next(self):
        self._k, sub = jax.random.split(self._k)
        return sub
    def normal(self, shape):
        return jax.random.normal(self._next(), shape, dtype=jnp.bfloat16)
    def randint(self, lo, hi, shape):
        return jax.random.randint(self._next(), shape, lo, hi, dtype=jnp.int32)
    def uniform(self, shape, lo=0.0, hi=1.0):
        return jax.random.uniform(self._next(), shape, jnp.bfloat16, lo, hi)
    def permutation(self, n):
        return jax.random.permutation(self._next(), n)


kernel_name = 'interleave_layers__sliding_local_dilated__glu_gated_bilinear__prompt'

def setup_inputs():
    _rng = _Rng(jax.random.key(int.from_bytes(__import__("os").urandom(4), "little")))
    _w = (lambda a: (lambda t: t.astype(jnp.bfloat16) if jnp.issubdtype(t.dtype, jnp.floating) else t)(jnp.asarray(a)))
    def _A_setup():
        B, S, D = 1, 2048, 576
        return {
            "x": _w((lambda *s: _rng.normal(s) * 0.05)(B, S, D)),
            "wqkv": _w((lambda *s: _rng.normal(s) * 0.05)(D, 3 * D)),
            "wo": _w((lambda *s: _rng.normal(s) * 0.05)(D, D)),
        }
    _A_in = _A_setup()

    def _B_setup():
        B, S, D, F = 1, 2048, 576, 4608
        return {
            "x": _w((lambda *s: _rng.normal(s) * 0.05)(B, S, D)),
            "w_gate": _w((lambda *s: _rng.normal(s) * 0.05)(D, F) * (D ** -0.5)),
            "w_up": _w((lambda *s: _rng.normal(s) * 0.05)(D, F) * (D ** -0.5)),
            "w_down": _w((lambda *s: _rng.normal(s) * 0.05)(F, D) * (F ** -0.5)),
        }
    _B_in = _B_setup()

    return {
        "A_x": _A_in["x"],
        "A_wqkv": _A_in["wqkv"],
        "A_wo": _A_in["wo"],
        "B_x": _B_in["x"],
        "B_w_gate": _B_in["w_gate"],
        "B_w_up": _B_in["w_up"],
        "B_w_down": _B_in["w_down"],
    }

def reference(A_x, A_wqkv, A_wo, B_x, B_w_gate, B_w_up, B_w_down):
    def _A_ref(x, wqkv, wo):
        B, S, D = x.shape
        H = 32; Dh = D // H
        W, dil = 8, 2
        qkv = (lambda x, *d: x.transpose(*d))((x @ wqkv).reshape(B, S, 3, H, Dh), 2, 0, 3, 1, 4)
        q, k, v = qkv[0], qkv[1], qkv[2]
        scale = Dh ** -0.5
        pos = jnp.arange(S)
        off = jnp.arange(W) * dil
        idx = pos[:, None] - off[None, :]
        mask = idx >= 0
        idx_c = jnp.where(mask, idx, 0).reshape(-1)
        kg = k[:, :, idx_c, :].reshape(B, H, S, W, Dh)
        vg = v[:, :, idx_c, :].reshape(B, H, S, W, Dh)
        logits = jnp.einsum("bhsd,bhswd->bhsw", q, kg) * scale
        logits = jnp.where(mask[None, None, :, :], logits, -1e9)
        attn = _softmax(logits, axis=-1)
        o = jnp.einsum("bhsw,bhswd->bhsd", attn, vg)
        return (lambda x, *d: x.transpose(*d))(o, 0, 2, 1, 3).reshape(B, S, D) @ wo

    def _B_ref(x, w_gate, w_up, w_down):
        g = jnp.einsum("bsd,df->bsf", x, w_gate)
        u = jnp.einsum("bsd,df->bsf", x, w_up)
        h = g * u
        return jnp.einsum("bsf,fd->bsd", h, w_down)

    x = A_x
    x = x + _A_ref(_layernorm(x, axis=-1), A_wqkv, A_wo)
    x = x + _B_ref(_layernorm(x, axis=-1), B_w_gate, B_w_up, B_w_down)
    x = x + _A_ref(_layernorm(x, axis=-1), A_wqkv, A_wo)
    x = x + _B_ref(_layernorm(x, axis=-1), B_w_gate, B_w_up, B_w_down)
    return x
```

```python
import functools
import jax, jax.numpy as jnp
from jax import lax
from jax.experimental import pallas as pl
from jax.experimental.pallas import tpu as pltpu

S, D, H, DH, F, W, DIL = 2048, 576, 32, 18, 4608, 8, 2
EPS = 1e-5
bf16, f32 = jnp.bfloat16, jnp.float32


def _ln(x):
    m = jnp.sum(x, axis=0, keepdims=True) * (1.0 / D)
    xc = x - m
    v = jnp.sum(xc * xc, axis=0, keepdims=True) * (1.0 / D)
    return xc * lax.rsqrt(v + EPS)


def _kernel(xT_hbm, wqkv_hbm, wo_hbm, wg_hbm, wu_hbm, wdT_hbm, out_hbm,
            xin, wqkv, wo, wg, wu, wd, wqkvT, woT, qkv, xa, xb, xh, xcb, ob, obuf, sem, osem,
            *, M, FC, split, qsplit, peel):
    NB = S // M
    NL = M // 128
    NC = F // FC

    x_cps = [pltpu.make_async_copy(xT_hbm.at[:, pl.ds(n * M, M)], xin.at[n], sem.at[n]) for n in range(NB)]
    w_cps = [pltpu.make_async_copy(s, d, sem.at[NB + i]) for i, (s, d) in enumerate(
        [(wqkv_hbm, wqkv), (wo_hbm, wo)])]
    f_cps = [[pltpu.make_async_copy(s.at[:, pl.ds(c * FC, FC)], d.at[:, pl.ds(c * FC, FC)], sem.at[NB + 2 + 3 * c + i])
              for i, (s, d) in enumerate([(wg_hbm, wg), (wu_hbm, wu), (wdT_hbm, wd)])] for c in range(NC)]
    x_cps[0].start()
    w_cps[0].start()
    x_cps[1].start()
    w_cps[1].start()
    for c in x_cps[2:]:
        c.start()
    for c in sum(f_cps, []):
        c.start()

    def stage_qkv(n, first_layer):
        m = n % NB
        if first_layer is True:
            x = xin[m].astype(f32)
        else:
            x = jnp.where(first_layer, xin[m].astype(f32), xcb[m])
        xa[n % 2] = x
        xn = _ln(x).astype(bf16)

        def mm():
            r = jnp.dot(wqkvT[...], xn, preferred_element_type=f32)
            for j in range(NL):
                qkv[(n % 3) * NL + j] = r[:, j * 128:(j + 1) * 128]
        return mm

    def stage_att(n):
        m = n % NB
        cur0, prv = (n % 3) * NL, ((n + 2) % 3) * NL + NL - 1
        lane = lax.broadcasted_iota(jnp.int32, (8, 128), 1)
        scale = DH ** -0.5
        for j in range(NL):
            ls = slice(None); cur = cur0 + j
            if j == 0:
                pslot, pls = prv, ls
                has_prev = m > 0
                sel = [None] + [jnp.logical_and(lane >= 128 - DIL * w, has_prev) for w in range(1, W)]
                valid = [None] + [jnp.logical_or(lane >= DIL * w, has_prev) for w in range(1, W)]
            else:
                pslot, pls = cur - 1, ls
                sel = [None] + [lane >= 128 - DIL * w for w in range(1, W)]
                valid = None

            def shifted(c, p, w):
                if w == 0:
                    return c
                return pltpu.roll(jnp.where(sel[w], p, c), DIL * w, 1)

            for hg in range(H // 8):
                rows = lambda part, d: pl.ds(part * D + hg * 8 * DH + d, 8, stride=DH)
                lg = [None] * W
                for d in range(DH):
                    q = qkv[cur, rows(0, d), ls]
                    kc = qkv[cur, rows(1, d), ls]
                    kp = qkv[pslot, rows(1, d), pls]
                    for w in range(W):
                        t = q * shifted(kc, kp, w)
                        lg[w] = t if d == 0 else lg[w] + t
                lg = [l * scale for l in lg]
                if valid is not None:
                    lg = [lg[0]] + [jnp.where(valid[w], lg[w], -1e9) for w in range(1, W)]
                mx = functools.reduce(jnp.maximum, lg)
                e = [jnp.exp(l - mx) for l in lg]
                r = 1.0 / functools.reduce(jnp.add, e)
                p = [x * r for x in e]
                for d in range(DH):
                    vc = qkv[cur, rows(2, d), ls]
                    vp = qkv[pslot, rows(2, d), pls]
                    o = None
                    for w in range(W):
                        t = p[w] * shifted(vc, vp, w)
                        o = t if o is None else o + t
                    ob[j, rows(0, d), ls] = o
                yield

    def stage_wo(n):
        x1 = xa[n % 2] + jnp.dot(woT[...], jnp.concatenate([ob[j].astype(bf16) for j in range(NL)], axis=1), preferred_element_type=f32)
        xb[n % 2] = x1
        xh[n % 2] = _ln(x1).T.astype(bf16)

    def stage_ffn(g, att=False, qk=False, waits=None):
        x = xh[g % 2]
        NU = NL * H // 8
        gen = stage_att(g + 1) if att else None
        acc = None
        for c in range(NC):
            if waits is not None:
                for cp in waits[c]:
                    cp.wait()
            if att and c < split:
                for _ in range(NU * (c + 1) // split - NU * c // split):
                    next(gen)
            if att and c == split:
                stage_wo(g + 1)
            if qk and c == qsplit - 1:
                mm = stage_qkv(g + 2, g + 2 < NB)
            if qk and c == qsplit:
                mm()
            cs = slice(c * FC, (c + 1) * FC)
            gg = jnp.dot(x, wg[:, cs], preferred_element_type=f32)
            uu = jnp.dot(x, wu[:, cs], preferred_element_type=f32)
            h = (gg * uu).astype(bf16)
            dd = lax.dot_general(wd[:, cs], h, (((1,), (1,)), ((), ())), preferred_element_type=f32)
            acc = dd if acc is None else acc + dd
        y = xb[g % 2] + acc
        xcb[g % NB] = y
        obuf[g % NB] = y.astype(bf16)

    def out_cp(m):
        return pltpu.make_async_copy(obuf.at[m], out_hbm.at[:, pl.ds(pl.multiple_of(m * M, M), M)], osem.at[m])

    w_cps[0].wait()
    for c in range(0, 3 * D, 128):
        wdt = min(128, 3 * D - c)
        wqkvT[c:c + wdt, :] = wqkv[:, c:c + wdt].astype(f32).T.astype(bf16)
    x_cps[0].wait()
    stage_qkv(0, True)()
    x_cps[1].wait()
    w_cps[1].wait()
    for c in range(0, D, 128):
        wdt = min(128, D - c)
        woT[c:c + wdt, :] = wo[:, c:c + wdt].astype(f32).T.astype(bf16)
    for _ in stage_att(0):
        pass
    stage_qkv(1, True)()
    stage_wo(0)
    for c in x_cps[2:]:
        c.wait()
    if not peel:
        for c in sum(f_cps, []):
            c.wait()

    def body(g, carry):
        stage_ffn(g, True, True)

        @pl.when(g >= NB)
        def _():
            out_cp(g - NB).start()
        return carry

    if peel:
        stage_ffn(0, True, True, f_cps)
    lax.fori_loop(int(peel), 2 * NB - 2, body, 0)
    g = 2 * NB - 2
    stage_ffn(g, True)
    out_cp(NB - 2).start()
    stage_ffn(g + 1)
    out_cp(NB - 1).start()
    for m in range(NB):
        out_cp(m).wait()


def make(M=256, FC=512, split=6, qsplit=8, peel=True, flags=None):
    NB = S // M
    V = pltpu.VMEM
    scratch = [
        V((NB, D, M), bf16), V((D, 3 * D), bf16), V((D, D), bf16), V((D, F), bf16), V((D, F), bf16), V((D, F), bf16),
        V((3 * D, D), bf16), V((D, D), bf16), V((3 * M // 128, 3 * D, 128), f32), V((2, D, M), f32), V((2, D, M), f32),
        V((2, M, D), bf16), V((NB, D, M), f32), V((M // 128, D, 128), f32), V((NB, D, M), bf16),
        pltpu.SemaphoreType.DMA((NB + 2 + 3 * (F // FC),)), pltpu.SemaphoreType.DMA((NB,)),
    ]

    def fn(A_x, A_wqkv, A_wo, B_x, B_w_gate, B_w_up, B_w_down):
        oT = pl.pallas_call(
            functools.partial(_kernel, M=M, FC=FC, split=split, qsplit=qsplit, peel=peel),
            in_specs=[pl.BlockSpec(memory_space=pl.ANY)] * 6,
            out_specs=pl.BlockSpec(memory_space=pl.ANY),
            out_shape=jax.ShapeDtypeStruct((D, S), bf16),
            scratch_shapes=scratch,
            compiler_params=pltpu.CompilerParams(vmem_limit_bytes=100 * 2**20, flags=flags),
            name=f"k2_{len(str(flags))}_{M}_{FC}_{split}_{qsplit}_{int(peel)}",
        )(A_x[0].T, A_wqkv, A_wo, B_w_gate, B_w_up, B_w_down.T)
        return oT.T[None]
    return fn


@jax.jit
def pallas_interleave_layers__sliding_local_dilated__glu_gated_bilinear__prompt_kernel(A_x, A_wqkv, A_wo, B_x, B_w_gate, B_w_up, B_w_down):
    fn = make(M=256, FC=768, split=4, qsplit=5, flags={"XLA_TPU_FORCE_LP_LLO_SCHEDULER": True})
    return fn(A_x, A_wqkv, A_wo, B_x, B_w_gate, B_w_up, B_w_down)
```
